```python
import jax
import jax.numpy as jnp

def _softmax(x, axis=-1):
    return jax.nn.softmax(x, axis=axis)
def _gelu(x):
    return jax.nn.gelu(x, approximate=True)
def _silu(x):
    return jax.nn.silu(x)
def _sigmoid(x):
    return jax.nn.sigmoid(x)
def _layernorm(x, axis=-1, eps=1e-5):
    m = jnp.mean(x, axis=axis, keepdims=True)
    v = jnp.var(x, axis=axis, keepdims=True)
    return (x - m) / jnp.sqrt(v + eps)
def _scatter_add(tgt, idx, src, axis=0):
    return tgt.at[idx].add(src)
def _segment_sum(src, seg, n):
    return jax.ops.segment_sum(src, seg, n)
class _Rng:
    def __init__(self, key):
        self._k = key
    def _next(self):
        self._k, sub = jax.random.split(self._k)
        return sub
    def normal(self, shape):
        return jax.random.normal(self._next(), shape, dtype=jnp.bfloat16)
    def randint(self, lo, hi, shape):
        return jax.random.randint(self._next(), shape, lo, hi, dtype=jnp.int32)
    def uniform(self, shape, lo=0.0, hi=1.0):
        return jax.random.uniform(self._next(), shape, jnp.bfloat16, lo, hi)
    def permutation(self, n):
        return jax.random.permutation(self._next(), n)


kernel_name = 'concat_heads__mha_block_cached__compressed_kv_cla__decode'

def setup_inputs():
    _rng = _Rng(jax.random.key(int.from_bytes(__import__("os").urandom(4), "little")))
    _w = (lambda a: (lambda t: t.astype(jnp.bfloat16) if jnp.issubdtype(t.dtype, jnp.floating) else t)(jnp.asarray(a)))
    def _A_setup():
        B, Sq, D = 4, 1, 576
        H, Sk, Dh = 32, 4096, 128
        return {
            "x": _w((lambda *s: _rng.normal(s) * 0.05)(B, Sq, D)),
            "k_cache": _w((lambda *s: _rng.normal(s) * 0.05)(B, H, Sk, Dh)),
            "v_cache": _w((lambda *s: _rng.normal(s) * 0.05)(B, H, Sk, Dh)),
            "wq": _w((lambda *s: _rng.normal(s) * 0.05)(D, H * Dh) * (D ** -0.5)),
            "wo": _w((lambda *s: _rng.normal(s) * 0.05)(H * Dh, D) * ((H * Dh) ** -0.5)),
        }
    _A_in = _A_setup()

    def _B_setup():
        B, H, Sq, Sk, D, M = 4, 32, 1, 4096, 128, 576
        Dc = 4 * D
        return {
            "x": _w((lambda *s: _rng.normal(s) * 0.05)(B, Sq, M)),
            "c_kv": _w((lambda *s: _rng.normal(s) * 0.05)(B, Sk, Dc)),
            "w_q": _w((lambda *s: _rng.normal(s) * 0.05)(M, H, D) * (M ** -0.5)),
            "w_uk": _w((lambda *s: _rng.normal(s) * 0.05)(Dc, H, D) * (Dc ** -0.5)),
            "w_uv": _w((lambda *s: _rng.normal(s) * 0.05)(Dc, H, D) * (Dc ** -0.5)),
            "w_o": _w((lambda *s: _rng.normal(s) * 0.05)(H, D, M) * ((H * D) ** -0.5)),
        }
    _B_in = _B_setup()

    return {
        "A_x": _A_in["x"],
        "A_k_cache": _A_in["k_cache"],
        "A_v_cache": _A_in["v_cache"],
        "A_wq": _A_in["wq"],
        "A_wo": _A_in["wo"],
        "B_x": _B_in["x"],
        "B_c_kv": _B_in["c_kv"],
        "B_w_q": _B_in["w_q"],
        "B_w_uk": _B_in["w_uk"],
        "B_w_uv": _B_in["w_uv"],
        "B_w_o": _B_in["w_o"],
    }

def reference(A_x, A_k_cache, A_v_cache, A_wq, A_wo, B_x, B_c_kv, B_w_q, B_w_uk, B_w_uv, B_w_o):
    def _A_ref(x, k_cache, v_cache, wq, wo):
        B, Sq, D = x.shape
        H, Dh = 32, 128
        q = (lambda x, *d: x.transpose(*d))((x @ wq).reshape(B, Sq, H, Dh), 0, 2, 1, 3)
        scores = jnp.einsum("bhqd,bhkd->bhqk", q, k_cache) * (Dh ** -0.5)
        p = _softmax(scores, axis=-1)
        o = jnp.einsum("bhqk,bhkd->bhqd", p, v_cache)
        return (lambda x, *d: x.transpose(*d))(o, 0, 2, 1, 3).reshape(B, Sq, H * Dh) @ wo

    def _B_ref(x, c_kv, w_q, w_uk, w_uv, w_o):
        B, Sq, M = x.shape[0], x.shape[1], x.shape[2]
        Sk = c_kv.shape[1]
        H, D = w_q.shape[1], w_q.shape[2]
        q = jnp.einsum("bqm,mhd->bhqd", x, w_q)
        k = jnp.einsum("bkc,chd->bhkd", c_kv, w_uk)
        v = jnp.einsum("bkc,chd->bhkd", c_kv, w_uv)
        scores = jnp.einsum("bhqd,bhkd->bhqk", q, k) * (D ** -0.5)
        off = Sk - Sq
        qi = jnp.arange(Sq)[:, None]
        kj = jnp.arange(Sk)[None, :]
        cmask = kj <= (qi + off)
        scores = jnp.where(cmask[None, None], scores, -1e9)
        p = _softmax(scores, axis=-1)
        ctx = jnp.einsum("bhqk,bhkd->bhqd", p, v)
        return jnp.einsum("bhqd,hdm->bqm", ctx, w_o)

    a = _A_ref(A_x, A_k_cache, A_v_cache, A_wq, A_wo)
    b = _B_ref(B_x, B_c_kv, B_w_q, B_w_uk, B_w_uv, B_w_o)
    return jnp.concatenate([a, b], axis=-1)
```

```python
import functools

import jax
import jax.numpy as jnp
from jax import lax
from jax.experimental import pallas as pl
from jax.experimental.pallas import tpu as pltpu

F32 = jnp.float32
BF16 = jnp.bfloat16
NT = (((1,), (1,)), ((), ()))

B, H, S, DH, M, DC = 4, 32, 4096, 128, 576, 512
NH = B * H
SUB = 128
PPH = S // SUB


def _dot(a, b):
    return jnp.dot(a, b, preferred_element_type=F32)


def _dot_nt(a, b):
    return lax.dot_general(a, b, NT, preferred_element_type=F32)


def make(HI=0, LAG=3, NB=4, NQK=2, NPV=2, WO_G=4, unroll_issue=True):
    LO = 1 - HI
    scale = DH ** -0.5

    def kernel(xa_h, k_h, v_h, wqa_h, woa_h, xb_h, c_h, wqb_h, wuk_h, wuv_h, wob_h,
               out_ref,
               xa_v, xb_v, kbuf, vbuf, wqa_v, woa_v, c_v, wqb_v, wuk_v, wuv_v, wob_v,
               q_s, o_s, e_s, qb_s, ql_s, s_s, cl_s, cx_s,
               sem_x, sem_k, sem_v, sem_w, sem_c, sem_oa, sem_ob):

        def start(src, dst, sem, prio):
            pltpu.make_async_copy(src, dst, sem).start(priority=prio)

        def wait_all(buf, sem):
            pltpu.make_async_copy(buf, buf, sem).wait()

        def wide(ref, j):
            r = pl.multiple_of((j // 4) * 16, 16)
            c = pl.multiple_of((j % 4) * 1024, 1024)
            return ref.at[pl.ds(r, 16), pl.ds(c, 1024)]

        def pair_wq(j):
            start(wide(wqa_h, j), wide(wqa_v, j), sem_w.at[0], HI)
            start(wqb_h.at[pl.ds(j * 4, 4)], wqb_v.at[pl.ds(j * 4, 4)], sem_w.at[1], LO)

        def pair_wu(j):
            start(wuk_h.at[pl.ds(j * 4, 4)], wuk_v.at[pl.ds(j * 4, 4)], sem_w.at[2], HI)
            start(wuv_h.at[pl.ds(j * 4, 4)], wuv_v.at[pl.ds(j * 4, 4)], sem_w.at[3], LO)

        def pair_c(b, j):
            r0 = pl.multiple_of(j * 32, 32)
            r1 = pl.multiple_of(j * 32 + S // 2, 32)
            start(c_h.at[b, pl.ds(r0, 32)], c_v.at[b, pl.ds(r0, 32)], sem_c.at[b], HI)
            start(c_h.at[b, pl.ds(r1, 32)], c_v.at[b, pl.ds(r1, 32)], sem_c.at[b], LO)

        def pair_kv(i, j):
            slot = i % NB
            r = j * SUB if isinstance(j, int) else pl.multiple_of(j * SUB, SUB)
            start(k_h.at[i, pl.ds(r, SUB)], kbuf.at[slot, pl.ds(r, SUB)], sem_k.at[slot], HI)
            start(v_h.at[i, pl.ds(r, SUB)], vbuf.at[slot, pl.ds(r, SUB)], sem_v.at[slot], LO)

        def pair_wo(j):
            start(wide(woa_h, j), wide(woa_v, j), sem_oa.at[j // 32], HI)
            r = pl.multiple_of(j * SUB, SUB)
            start(wob_h.at[pl.ds(r, SUB)], wob_v.at[pl.ds(r, SUB)],
                  sem_ob.at[j // (WO_G * M // SUB)], LO)

        def run(pair, j0, n):
            def body(t, c):
                pair(j0 + t)
                return c
            lax.fori_loop(0, n, body, 0)

        start(xa_h, xa_v, sem_x.at[0], HI)
        start(xb_h, xb_v, sem_x.at[1], HI)
        run(pair_wq, 0, 40)
        e_s[...] = (lax.broadcasted_iota(jnp.int32, (128, 2048), 1) // 16
                    == lax.broadcasted_iota(jnp.int32, (128, 2048), 0)).astype(F32).astype(BF16)
        o_s[...] = jnp.zeros(o_s.shape, F32)
        run(pair_wq, 40, 104)
        run(pair_wu, 0, 64)

        def diag16(t):
            keep = (lax.broadcasted_iota(jnp.int32, t.shape, 0) % 16
                    == lax.broadcasted_iota(jnp.int32, t.shape, 1) % 16)
            return jnp.where(keep, t, 0.0).astype(BF16)

        def wslab(ref, m0, n, g):
            return ref[pl.ds(m0, n), pl.ds(16 * g, 16), :].reshape(n * 16, DH)

        wait_all(xa_v, sem_x.at[0])
        wait_all(wqa_v, sem_w.at[0])
        xa = xa_v[...].astype(F32)
        xa8 = jnp.concatenate([xa, xa], axis=0).astype(BF16)
        for j in range(4):
            qa = _dot(xa8, wqa_v[:, 1024 * j:1024 * (j + 1)])
            for h in range(8):
                q_s[8 * j + h] = qa[:, 128 * h:128 * (h + 1)]
            run(pair_wu, 64 + 6 * j, 6)

        wait_all(xb_v, sem_x.at[1])
        wait_all(wqb_v, sem_w.at[1])
        xb = xb_v[...].astype(F32)
        xr = jnp.concatenate([jnp.broadcast_to(xb[b:b + 1], (16, M)) for b in range(B)],
                             axis=0).astype(BF16)
        qb = [None, None]
        for j in range(5):
            n = min(128, M - 128 * j)
            lj = diag16(_dot(xr[:, 128 * j:128 * j + n], e_s[:n, :16 * n]))
            for g in range(2):
                t = _dot(lj, wslab(wqb_v, 128 * j, n, g))
                qb[g] = t if j == 0 else qb[g] + t
            run(pair_wu, 88 + 8 * j, 8)
        for g in range(2):
            qb_s[g] = qb[g].astype(BF16)

        run(functools.partial(pair_c, 0), 0, 8)
        wait_all(wuk_v, sem_w.at[2])

        def ql_body(j, c):
            m0 = pl.multiple_of(j * 128, 128)
            for g in range(2):
                t = diag16(_dot_nt(qb_s[g], wslab(wuk_v, m0, 128, g)))
                ql_s[j, g] = _dot_nt(t, e_s[...]).astype(BF16)
                run(functools.partial(pair_c, 0), 8 + 14 * j + 7 * g, 7)
            return c
        lax.fori_loop(0, 4, ql_body, 0)
        run(functools.partial(pair_c, 1), 0, 64)

        def attn_issue(b, step):
            @pl.when(b < 2)
            def _():
                run(functools.partial(pair_c, b + 2), 4 * step, 4)

            @pl.when(b >= 2)
            def _():
                run(functools.partial(pair_kv, b - 2), 2 * step, 2)

        def attn_body(b, c):
            r = pl.multiple_of(b * 16, 16)
            ql = jnp.concatenate(
                [jnp.concatenate([ql_s[j, g, pl.ds(r, 16), :] for j in range(4)], axis=1)
                 for g in range(2)], axis=0)
            wait_all(c_v.at[b], sem_c.at[b])

            def qk(t, m):
                k0 = pl.multiple_of(t * 512, 512)
                s = _dot_nt(ql, c_v[b, pl.ds(k0, 512), :]) * scale
                s_s[t] = s
                attn_issue(b, t)
                return jnp.maximum(m, s)
            m = lax.fori_loop(0, 8, qk, jnp.full((32, 512), -jnp.inf, F32))
            m = jnp.max(m, axis=1, keepdims=True)

            def pv(t, carry):
                l, acc = carry
                k0 = pl.multiple_of(t * 512, 512)
                p = jnp.exp(s_s[t] - m)
                acc = acc + _dot(p.astype(BF16), c_v[b, pl.ds(k0, 512), :])
                attn_issue(b, 8 + t)
                return l + p, acc
            l, acc = lax.fori_loop(0, 8, pv, (jnp.zeros((32, 512), F32), jnp.zeros((32, 512), F32)))
            ctx = (acc / jnp.sum(l, axis=1, keepdims=True)).astype(BF16)
            for g in range(2):
                for j in range(4):
                    cl_s[j, g, pl.ds(r, 16), :] = ctx[16 * g:16 * (g + 1), 128 * j:128 * (j + 1)]
            return c
        lax.fori_loop(0, B, attn_body, 0)

        wait_all(wuv_v, sem_w.at[3])

        def cx_body(j, carry):
            m0 = pl.multiple_of(j * 128, 128)
            out = []
            for g in range(2):
                lj = diag16(_dot(cl_s[j, g], e_s[...]))
                out.append(carry[g] + _dot(lj, wslab(wuv_v, m0, 128, g)))
                run(functools.partial(pair_kv, 2), 8 * j + 4 * g, 4)
            return tuple(out)
        cx = lax.fori_loop(0, 4, cx_body, (jnp.zeros((64, DH), F32), jnp.zeros((64, DH), F32)))
        cx = jnp.concatenate(cx, axis=0).astype(BF16)
        ro = lax.broadcasted_iota(jnp.int32, (256, 128), 0)
        co = lax.broadcasted_iota(jnp.int32, (256, 128), 1)
        hd, bb = ro // 8, ro % 8
        perm = jnp.where((co == (hd // 16) * 64 + bb * 16 + hd % 16) & (bb < B), 1.0, 0.0).astype(BF16)
        cx_s[...] = _dot(perm, cx).reshape(H, 8, DH)
        for i in range(3, LAG):
            run(functools.partial(pair_kv, i), 0, PPH)

        def head(i, issue):
            slot = i % NB
            b, h = i // H, i % H
            q = jnp.broadcast_to(q_s[h, pl.ds(b, 1), :], (8, DH)).astype(BF16)
            wait_all(kbuf.at[slot], sem_k.at[slot])
            ss = []
            for t in range(NQK):
                n = S // NQK
                ss.append(_dot_nt(q, kbuf[slot, t * n:(t + 1) * n, :]))
                issue(t)
            s = jnp.concatenate(ss, axis=1) * scale
            p = jnp.exp(s - jnp.max(s, axis=1, keepdims=True))
            l = jnp.sum(p, axis=1, keepdims=True)
            p = p.astype(BF16)
            wait_all(vbuf.at[slot], sem_v.at[slot])
            acc = None
            for t in range(NPV):
                n = S // NPV
                d = _dot(p[:, t * n:(t + 1) * n], vbuf[slot, t * n:(t + 1) * n, :])
                acc = d if acc is None else acc + d
                issue(NQK + t)
            o_s[h, pl.ds(b, 1), :] = (acc / l)[0:1]

        per = PPH // (NQK + NPV)

        def main_body(i, c):
            def issue(t):
                if unroll_issue:
                    for j in range(per * t, per * (t + 1)):
                        pair_kv(i + LAG, j)
                else:
                    run(functools.partial(pair_kv, i + LAG), per * t, per)
            head(i, issue)
            return c
        lax.fori_loop(0, NH - LAG, main_body, 0)

        per_t = 96 // LAG // (NQK + NPV)

        def tail_body(i, c):
            head(i, lambda t: run(pair_wo, ((i - (NH - LAG)) * (NQK + NPV) + t) * per_t, per_t))
            return c
        lax.fori_loop(NH - LAG, NH, tail_body, 0)
        done = per_t * LAG * (NQK + NPV)

        oa = jnp.concatenate([o_s[h] for h in range(H)], axis=1).astype(BF16)
        ya = []
        for j in range(5):
            n = min(128, M - 128 * j)
            wait_all(woa_v.at[pl.ds(128 * j, n)], sem_oa.at[j])
            ya.append(_dot_nt(oa, woa_v[128 * j:128 * j + n, :]))
            if j < 2:
                step = (144 - done) // 2
                run(pair_wo, done + step * j, step)
        ya = jnp.concatenate(ya, axis=1)

        def yb_body(gi, acc):
            r0 = pl.multiple_of(gi * (WO_G * M), WO_G * M)
            wait_all(wob_v.at[pl.ds(r0, WO_G * M)], sem_ob.at[gi])
            for t in range(WO_G):
                acc = acc + _dot_nt(cx_s[gi * WO_G + t].astype(BF16),
                                    wob_v[pl.ds(pl.multiple_of(r0 + t * M, 64), M), :])
            return acc
        yb = lax.fori_loop(0, H // WO_G, yb_body, jnp.zeros((8, M), F32))
        out_ref[...] = jnp.concatenate([ya, yb], axis=1)[0:B].astype(out_ref.dtype)

    def fn(A_x, A_k_cache, A_v_cache, A_wq, A_wo, B_x, B_c_kv, B_w_q, B_w_uk, B_w_uv, B_w_o):
        any_spec = pl.BlockSpec(memory_space=pl.ANY)
        out = pl.pallas_call(
            kernel,
            in_specs=[any_spec] * 11,
            out_specs=pl.BlockSpec(memory_space=pltpu.VMEM),
            out_shape=jax.ShapeDtypeStruct((B, 2 * M), BF16),
            scratch_shapes=[
                pltpu.VMEM((B, M), BF16), pltpu.VMEM((B, M), BF16),
                pltpu.VMEM((NB, S, DH), BF16), pltpu.VMEM((NB, S, DH), BF16),
                pltpu.VMEM((M, H * DH), BF16), pltpu.VMEM((M, H * DH), BF16),
                pltpu.VMEM((B, S, DC), BF16),
                pltpu.VMEM((M, H, DH), BF16), pltpu.VMEM((DC, H, DH), BF16),
                pltpu.VMEM((DC, H, DH), BF16), pltpu.VMEM((H * M, DH), BF16),
                pltpu.VMEM((H, 8, DH), F32), pltpu.VMEM((H, 8, DH), F32),
                pltpu.VMEM((128, 2048), BF16), pltpu.VMEM((2, 64, DH), BF16),
                pltpu.VMEM((4, 2, 64, 128), BF16), pltpu.VMEM((8, 32, 512), F32),
                pltpu.VMEM((4, 2, 64, 128), BF16), pltpu.VMEM((H, 8, DH), F32),
                pltpu.SemaphoreType.DMA((2,)), pltpu.SemaphoreType.DMA((NB,)),
                pltpu.SemaphoreType.DMA((NB,)), pltpu.SemaphoreType.DMA((4,)),
                pltpu.SemaphoreType.DMA((B,)), pltpu.SemaphoreType.DMA((5,)),
                pltpu.SemaphoreType.DMA((H // WO_G,)),
            ],
            compiler_params=pltpu.CompilerParams(vmem_limit_bytes=100 * 1024 * 1024),
        )(
            A_x.reshape(B, M),
            A_k_cache.reshape(NH, S, DH),
            A_v_cache.reshape(NH, S, DH),
            A_wq,
            A_wo.T,
            B_x.reshape(B, M),
            B_c_kv,
            B_w_q,
            B_w_uk,
            B_w_uv,
            B_w_o.transpose(0, 2, 1).reshape(H * M, DH),
        )
        return out.reshape(B, 1, 2 * M)

    return fn


_impl = make(**dict(unroll_issue=False))


@jax.jit
def pallas_concat_heads__mha_block_cached__compressed_kv_cla__decode_kernel(
    A_x, A_k_cache, A_v_cache, A_wq, A_wo, B_x, B_c_kv, B_w_q, B_w_uk, B_w_uv, B_w_o,
):
    return _impl(A_x, A_k_cache, A_v_cache, A_wq, A_wo, B_x, B_c_kv, B_w_q, B_w_uk, B_w_uv, B_w_o)
```

```python
import jax
import jax.numpy as jnp
from jax import lax
from jax.experimental import pallas as pl
from jax.experimental.pallas import tpu as pltpu

F32 = jnp.float32
BF16 = jnp.bfloat16
NT = (((1,), (1,)), ((), ()))

B, H, S, DH, M, DC = 4, 32, 4096, 128, 576, 512
NH = B * H
GH = 8
NG = 3
SEG = 64
RPG = S // SEG
RPH = RPG // GH


def _dot(a, b):
    return jnp.dot(a, b, preferred_element_type=F32)


def _dot_nt(a, b):
    return lax.dot_general(a, b, NT, preferred_element_type=F32)


class _Scopes:
    def __init__(self, on):
        self.cur = None
        self.on = on

    def __call__(self, name):
        if not self.on:
            return
        if self.cur is not None:
            self.cur.__exit__(None, None, None)
        self.cur = None
        if name is not None:
            self.cur = jax.named_scope(name)
            self.cur.__enter__()


def make(NQK=1, NPV=1, scopes=False, nobc=True, nosc=True, LAG=10, WOA_H=8, WOB0=12, WOB1=2):
    scale = DH ** -0.5

    def kernel(xa_h, k_h, v_h, wqa_h, woa_h, xb_h, c_h, wqb_h, wuk_h, wuv_h, wob_h,
               out_ref,
               xa_v, xb_v, kbuf, vbuf, wqa_v, woa_v, c_v, wqb_v, wuk_v, wuv_v, wob_v,
               q_s, o_s, e_s, qb_s, ql_s, s_s, cl_s, cx_s,
               sem_x, sem_k, sem_v, sem_w, sem_ob):

        def start(hbm, vmem, idx, sem, thread):
            pltpu.make_async_copy(hbm.at[idx], vmem.at[idx], sem).start(priority=thread)

        def wait_all(buf, sem):
            pltpu.make_async_copy(buf, buf, sem).wait()

        def wide(d, t):
            r = pl.multiple_of((t >> 2) * 8, 8)
            c = pl.multiple_of((t & 3) * 1024, 1024)
            return (pl.ds(3 * d, 3), pl.ds(r, 8), pl.ds(c, 1024))

        def round_wq(t):
            for d in range(3):
                start(wqa_h, wqa_v, wide(d, t), sem_w.at[0], 0)
                start(wqb_h, wqb_v, (pl.ds(3 * d, 3), pl.ds(2 * t, 2)), sem_w.at[1], 1)

        def round_wu(t):
            for u in range(2):
                for d in range(2):
                    idx = (pl.ds(2 * d, 2), pl.ds(2 * t + 64 * u, 2))
                    start(wuk_h, wuk_v, idx, sem_w.at[2], 0)
                    start(wuv_h, wuv_v, idx, sem_w.at[3], 1)

        def round_c(t):
            r = pl.multiple_of(t * 16, 16)
            for d in range(4):
                for w in range(2):
                    start(c_h, c_v, (pl.ds(8 * w + 2 * d, 2), pl.ds(r, 16)), sem_w.at[4], w)

        def rounds_kv(t0, n):
            g = t0 // RPG if isinstance(t0, int) else t0 >> 6
            slot = g % NG if isinstance(g, int) else lax.rem(g, NG)

            def one(t):
                rows = pl.ds(pl.multiple_of((t & (RPG - 1)) * SEG, SEG), SEG)
                for d in range(GH // 2):
                    for hbm, buf, sem, w in ((k_h, kbuf, sem_k, 0), (v_h, vbuf, sem_v, 1)):
                        pltpu.make_async_copy(hbm.at[pl.ds(g * GH + 2 * d, 2), rows],
                                              buf.at[slot, pl.ds(2 * d, 2), rows],
                                              sem.at[slot]).start(priority=w)
            run(one, t0, n)

        def round_woa(t):
            for u in range(2):
                for d in range(3):
                    start(woa_h, woa_v, wide(d, 2 * t + u), sem_w.at[5], (3 * u + d) % 2)

        def round_wob(t):
            g = lax.div(t, 3)
            for u in range(3):
                rows = pl.ds(pl.multiple_of((t - 3 * g) * 192 + 64 * u, 64), 64)
                for w in range(2):
                    pltpu.make_async_copy(wob_h.at[pl.ds(2 * w, 2), g, rows],
                                          wob_v.at[g, pl.ds(2 * w, 2), rows],
                                          sem_ob.at[g]).start(priority=w)

        def run(fn, t0, n):
            def body(t, c):
                fn(t0 + t)
                return c
            lax.fori_loop(0, n, body, 0)

        sc = _Scopes(scopes)
        sc("p0_prologue")
        run(round_wq, 0, 14)
        pltpu.make_async_copy(xa_h, xa_v, sem_x.at[0]).start(priority=0)
        pltpu.make_async_copy(xb_h, xb_v, sem_x.at[1]).start(priority=1)
        e_s[...] = ((lax.broadcasted_iota(jnp.int32, (128, 2048), 1) >> 4)
                    == lax.broadcasted_iota(jnp.int32, (128, 2048), 0)).astype(F32).astype(BF16)
        o_s[...] = jnp.zeros(o_s.shape, F32)
        run(round_wq, 14, 18)
        run(round_wu, 0, 24)

        def diag16(t):
            keep = ((lax.broadcasted_iota(jnp.int32, t.shape, 0) & 15)
                    == (lax.broadcasted_iota(jnp.int32, t.shape, 1) & 15))
            return jnp.where(keep, t, 0.0).astype(BF16)

        def heads16(g):
            return pl.ds(16 * g, 16)

        sc("p1_qa")
        wait_all(xa_v, sem_x.at[0])
        wait_all(wqa_v, sem_w.at[0])
        xa = xa_v[...].astype(F32)
        xa8 = jnp.concatenate([xa, xa], axis=0).astype(BF16)

        def qa_body(j, c):
            w = wqa_v[:, :, pl.ds(pl.multiple_of(j * 1024, 1024), 1024)].reshape(M, 1024)
            qa = _dot(xa8, w)
            for h in range(8):
                q_s[8 * j + h] = qa[:, 128 * h:128 * (h + 1)]
            run(round_wu, 24 + 2 * j, 2)
            return c
        lax.fori_loop(0, 4, qa_body, 0)

        sc("p2_qb")
        wait_all(xb_v, sem_x.at[1])
        wait_all(wqb_v, sem_w.at[1])
        xb = xb_v[...].astype(F32)
        xr = jnp.concatenate([jnp.broadcast_to(xb[b:b + 1], (16, M)) for b in range(B)],
                             axis=0).astype(BF16)
        for j in range(4):
            cl_s[j, 0] = xr[:, 128 * j:128 * (j + 1)]
        lj = diag16(_dot(xr[:, 512:M], e_s[:64, :1024]))
        qb = tuple(_dot(lj, wqb_v[8, :, heads16(g), :].reshape(1024, DH)) for g in range(2))
        run(round_c, 0, 8)

        def qb_body(j, carry):
            lj = diag16(_dot(cl_s[j, 0], e_s[...]))
            out = []
            for g in range(2):
                w = wqb_v[pl.ds(2 * j, 2), :, heads16(g), :].reshape(2048, DH)
                out.append(carry[g] + _dot(lj, w))
                run(round_c, 8 + 6 * j + 3 * g, 3)
            return tuple(out)
        qb = lax.fori_loop(0, 4, qb_body, qb)
        for g in range(2):
            qb_s[g] = qb[g].astype(BF16)

        sc("p3_ql")
        wait_all(wuk_v, sem_w.at[2])

        def ql_body(j, c):
            for g in range(2):
                t = diag16(_dot_nt(qb_s[g], wuk_v[j, :, heads16(g), :].reshape(2048, DH)))
                run(round_c, 32 + 8 * j + 4 * g, 2)
                ql_s[j, g] = _dot_nt(t, e_s[...]).astype(BF16)
                run(round_c, 34 + 8 * j + 4 * g, 2)
            return c
        lax.fori_loop(0, 4, ql_body, 0)

        sc("p5_attn")
        rounds_kv(0, 16)
        wait_all(c_v, sem_w.at[4])

        def attn_body(b, c):
            r = pl.multiple_of(b * 16, 16)
            ql = jnp.concatenate(
                [jnp.concatenate([ql_s[j, g, pl.ds(r, 16), :] for j in range(4)], axis=1)
                 for g in range(2)], axis=0)

            def qk(t, m):
                s = _dot_nt(ql, c_v[4 * b + t]) * scale
                s_s[t] = s
                for u in range(8):
                    m = jnp.maximum(m, s[:, 128 * u:128 * (u + 1)])
                rounds_kv(16 + 12 * b + 2 * t, 2)
                return m
            m = lax.fori_loop(0, 4, qk, jnp.full((32, 128), -jnp.inf, F32))
            m = jnp.max(m, axis=1, keepdims=True)

            def pv(t, carry):
                l, acc = carry
                p = jnp.exp(s_s[t] - m)
                acc = acc + _dot(p.astype(BF16), c_v[4 * b + t])
                for u in range(8):
                    l = l + p[:, 128 * u:128 * (u + 1)]
                rounds_kv(24 + 12 * b + t, 1)
                return l, acc
            l, acc = lax.fori_loop(0, 4, pv, (jnp.zeros((32, 128), F32), jnp.zeros((32, DC), F32)))
            ctx = (acc / jnp.sum(l, axis=1, keepdims=True)).astype(BF16)
            for g in range(2):
                for j in range(4):
                    cl_s[j, g, pl.ds(r, 16), :] = ctx[16 * g:16 * (g + 1), 128 * j:128 * (j + 1)]
            return c
        lax.fori_loop(0, B, attn_body, 0)

        sc("p6_cx")
        wait_all(wuv_v, sem_w.at[3])

        def cx_body(j, carry):
            out = []
            for g in range(2):
                lj = diag16(_dot(cl_s[j, g], e_s[...]))
                out.append(carry[g] + _dot(lj, wuv_v[j, :, heads16(g), :].reshape(2048, DH)))
                rounds_kv(64 + 4 * j + 2 * g, 2)
            return tuple(out)
        cx = lax.fori_loop(0, 4, cx_body, (jnp.zeros((64, DH), F32), jnp.zeros((64, DH), F32)))
        cx = jnp.concatenate(cx, axis=0).astype(BF16)
        ro = lax.broadcasted_iota(jnp.int32, (256, 128), 0)
        co = lax.broadcasted_iota(jnp.int32, (256, 128), 1)
        hd, bb = ro >> 3, ro & 7
        perm = jnp.where((co == (hd >> 4) * 64 + bb * 16 + (hd & 15)) & (bb < B), 1.0, 0.0).astype(BF16)
        cx_s[...] = _dot(perm, cx).reshape(H, 8, DH)
        if LAG > 10:
            rounds_kv(80, RPH * (LAG - 10))

        sc("p7_main")
        NI = NQK + NPV
        per = RPH // NI
        per_a = 16 // WOA_H // NI
        per_b = WOB0 // (LAG - WOA_H) // NI
        assert per_a * WOA_H * NI == 16 and per_b * (LAG - WOA_H) * NI == WOB0

        def head(i, c):
            def issue(t):
                @pl.when(i < NH - LAG)
                def _():
                    rounds_kv((i + LAG) * RPH + per * t, per)

                @pl.when(i >= NH - LAG)
                def _():
                    @pl.when(i < NH - LAG + WOA_H)
                    def _():
                        run(round_woa, ((i - (NH - LAG)) * NI + t) * per_a, per_a)

                    @pl.when(i >= NH - LAG + WOA_H)
                    def _():
                        run(round_wob, ((i - (NH - LAG + WOA_H)) * NI + t) * per_b, per_b)

            slot = lax.rem(i >> 3, NG)
            hh = i & (GH - 1)
            b, h = i >> 5, i & (H - 1)

            @pl.when(hh == 0)
            def _():
                wait_all(kbuf.at[slot], sem_k.at[slot])
                wait_all(vbuf.at[slot], sem_v.at[slot])

            q = jnp.broadcast_to(q_s[h, pl.ds(b, 1), :], (8, DH)).astype(BF16)
            ss = []
            for t in range(NQK):
                n = S // NQK
                ss.append(_dot_nt(q, kbuf[slot, hh, t * n:(t + 1) * n, :]))
                issue(t)
            s = jnp.concatenate(ss, axis=1) * scale
            p = jnp.exp(s - jnp.max(s, axis=1, keepdims=True))
            l = jnp.sum(p, axis=1, keepdims=True)
            p = p.astype(BF16)
            acc = None
            for t in range(NPV):
                n = S // NPV
                d = _dot(p[:, t * n:(t + 1) * n], vbuf[slot, hh, t * n:(t + 1) * n, :])
                acc = d if acc is None else acc + d
                if t == NPV - 1:
                    o_s[h, pl.ds(b, 1), :] = (acc / l)[0:1]
                issue(NQK + t)
            return c
        lax.fori_loop(0, NH, head, 0)

        sc("p8_ya")
        run(round_wob, WOB0, 24 - WOB0 - 4 * WOB1)
        oa = jnp.concatenate([o_s[h] for h in range(H)], axis=1).astype(BF16)
        wait_all(woa_v, sem_w.at[5])

        def ya_body(j, c):
            q_s[j] = _dot_nt(oa, woa_v[pl.ds(2 * j, 2)].reshape(128, H * DH))
            if WOB1:
                run(round_wob, 24 - 4 * WOB1 + WOB1 * j, WOB1)
            return c
        lax.fori_loop(0, 4, ya_body, 0)
        ya = jnp.concatenate([q_s[j] for j in range(4)] + [_dot_nt(oa, woa_v[8])], axis=1)

        sc("p9_yb")

        def yb_body(g, acc):
            wait_all(wob_v.at[g], sem_ob.at[g])
            for t in range(4):
                acc = acc + _dot_nt(cx_s[g + 8 * t].astype(BF16), wob_v[g, t])
            return acc
        yb = lax.fori_loop(0, 8, yb_body, jnp.zeros((8, M), F32))
        out_ref[...] = jnp.concatenate([ya, yb], axis=1)[0:B].astype(out_ref.dtype)
        sc(None)

    def fn(A_x, A_k_cache, A_v_cache, A_wq, A_wo, B_x, B_c_kv, B_w_q, B_w_uk, B_w_uv, B_w_o):
        any_spec = pl.BlockSpec(memory_space=pl.ANY)
        out = pl.pallas_call(
            kernel,
            in_specs=[any_spec] * 11,
            out_specs=pl.BlockSpec(memory_space=pltpu.VMEM),
            out_shape=jax.ShapeDtypeStruct((B, 2 * M), BF16),
            scratch_shapes=[
                pltpu.VMEM((B, M), BF16), pltpu.VMEM((B, M), BF16),
                pltpu.VMEM((NG, GH, S, DH), BF16), pltpu.VMEM((NG, GH, S, DH), BF16),
                pltpu.VMEM((9, 64, H * DH), BF16), pltpu.VMEM((9, 64, H * DH), BF16),
                pltpu.VMEM((16, 1024, DC), BF16),
                pltpu.VMEM((9, 64, H, DH), BF16), pltpu.VMEM((4, 128, H, DH), BF16),
                pltpu.VMEM((4, 128, H, DH), BF16), pltpu.VMEM((8, 4, M, DH), BF16),
                pltpu.VMEM((H, 8, DH), F32), pltpu.VMEM((H, 8, DH), F32),
                pltpu.VMEM((128, 2048), BF16), pltpu.VMEM((2, 64, DH), BF16),
                pltpu.VMEM((4, 2, 64, 128), BF16), pltpu.VMEM((4, 32, 1024), F32),
                pltpu.VMEM((4, 2, 64, 128), BF16), pltpu.VMEM((H, 8, DH), F32),
                pltpu.SemaphoreType.DMA((2,)), pltpu.SemaphoreType.DMA((NG,)),
                pltpu.SemaphoreType.DMA((NG,)), pltpu.SemaphoreType.DMA((6,)),
                pltpu.SemaphoreType.DMA((8,)),
            ],
            compiler_params=pltpu.CompilerParams(vmem_limit_bytes=110 * 1024 * 1024,
                                                 disable_bounds_checks=nobc,
                                                 disable_semaphore_checks=nosc),
        )(
            A_x.reshape(B, M),
            A_k_cache.reshape(NH, S, DH),
            A_v_cache.reshape(NH, S, DH),
            A_wq.reshape(9, 64, H * DH),
            A_wo.T.reshape(9, 64, H * DH),
            B_x.reshape(B, M),
            B_c_kv.reshape(16, 1024, DC),
            B_w_q.reshape(9, 64, H, DH),
            B_w_uk.reshape(4, 128, H, DH),
            B_w_uv.reshape(4, 128, H, DH),
            B_w_o.transpose(0, 2, 1).reshape(4, 8, M, DH),
        )
        return out.reshape(B, 1, 2 * M)

    return fn


_impl = make(**dict(WOA_H=4,WOB0=12))


@jax.jit
def pallas_concat_heads__mha_block_cached__compressed_kv_cla__decode_kernel(
    A_x, A_k_cache, A_v_cache, A_wq, A_wo, B_x, B_c_kv, B_w_q, B_w_uk, B_w_uv, B_w_o,
):
    return _impl(A_x, A_k_cache, A_v_cache, A_wq, A_wo, B_x, B_c_kv, B_w_q, B_w_uk, B_w_uv, B_w_o)
```

```python
import functools

import jax
import jax.numpy as jnp
from jax import lax
from jax.experimental import pallas as pl
from jax.experimental.pallas import tpu as pltpu

F32 = jnp.float32
BF16 = jnp.bfloat16

B, H, S, DH, M, DC = 4, 32, 4096, 128, 576, 512
GH = 8
NGRP = B * H // GH
SCALE = DH ** -0.5

KV_ROUNDS = (8, 5, 2)
WO_ROUNDS = (6, 4, 2)
WO_EARLY = WO_ROUNDS[0] + GH * (WO_ROUNDS[1] + WO_ROUNDS[2])


def _dot(a, b):
    return jnp.dot(a, b, preferred_element_type=F32)


def _dot_nt(a, b):
    return lax.dot_general(a, b, (((1,), (1,)), ((), ())), preferred_element_type=F32)


def _iota(shape, axis):
    return lax.broadcasted_iota(jnp.int32, shape, axis)


def _diag16(t):
    keep = (_iota(t.shape, 0) & 15) == (_iota(t.shape, 1) & 15)
    return jnp.where(keep, t, 0.0).astype(BF16)


def _heads16(g):
    return pl.ds(16 * g, 16)


def _start(src, dst, sem, thread):
    pltpu.make_async_copy(src, dst, sem).start(priority=thread)


def _wait_all(buf, sem):
    pltpu.make_async_copy(buf, buf, sem).wait()


def _run(round_fn, t0, n):
    def body(t, c):
        round_fn(t0 + t)
        return c
    lax.fori_loop(0, n, body, 0)


def _stream(xa_h, k_h, v_h, wqa_h, woa_h, xb_h, c_h, wqb_h, wuk_h, wuv_h, wob_h,
            out_ref,
            xa_v, xb_v, kbuf, vbuf, wqa_v, woa_v, c_v, wqb_v, wuk_v, wuv_v, wob_v,
            q_s, o_s, sa_s, e_s, qb_s, ql_s, sb_s, cl_s, cx_s,
            sem_x, sem_k, sem_v, sem_w, sem_c, sem_oa, sem_ob):

    def round_wq(t, thread=0):
        r = pl.multiple_of((t >> 2) * 8, 8)
        c = pl.multiple_of((t & 3) * 1024, 1024)
        for d in range(3):
            ia = (pl.ds(3 * d, 3), pl.ds(r, 8), pl.ds(c, 1024))
            ib = (pl.ds(3 * d, 3), pl.ds(2 * t, 2))
            _start(wqa_h.at[ia], wqa_v.at[ia], sem_w.at[0], thread)
            _start(wqb_h.at[ib], wqb_v.at[ib], sem_w.at[1], 1)

    def round_wu(t):
        for u in range(2):
            for d in range(2):
                i = (pl.ds(2 * d, 2), pl.ds(2 * t + 64 * u, 2))
                _start(wuk_h.at[i], wuk_v.at[i], sem_w.at[2], 0)
                _start(wuv_h.at[i], wuv_v.at[i], sem_w.at[3], 1)

    def round_c(t):
        r = pl.multiple_of(t * 16, 16)
        for d in range(4):
            for w in range(2):
                i = (pl.ds(8 * w + 2 * d, 2), pl.ds(r, 16))
                _start(c_h.at[i], c_v.at[i], sem_c.at[2 * w + d // 2], w)

    def round_kv(g, t):
        rows = pl.ds(pl.multiple_of(t * 64, 64), 64)
        for d in range(GH // 2):
            hs = pl.ds(2 * d, 2)
            _start(k_h.at[g, hs, rows], kbuf.at[g & 1, hs, rows], sem_k.at[g & 1], 0)
            _start(v_h.at[g, hs, rows], vbuf.at[g & 1, hs, rows], sem_v.at[g & 1], 1)

    def round_wo(t, last=False):
        g = lax.div(t, 9)
        rows = pl.ds(pl.multiple_of((t - 9 * g) * 64, 64), 64)
        for w in range(2):
            hs = pl.ds(2 * w, 2)
            _start(wob_h.at[hs, g, rows], wob_v.at[g, hs, rows], sem_ob.at[g], 0)
            cols = pl.ds(pl.multiple_of((t & 1) * 2048 + w * 1024, 1024), 1024)
            if last:
                i = (8, pl.ds(pl.multiple_of(((t >> 1) & 3) * 16, 16), 16), cols)
            else:
                r = pl.multiple_of(((t >> 1) & 7) * 8, 8)
                i = (pl.ds(2 * (t >> 4), 2), pl.ds(r, 8), cols)
            _start(woa_h.at[i], woa_v.at[i], sem_oa.at[t >> 4], 1)

    round_kv0 = functools.partial(round_kv, 0)

    _run(functools.partial(round_wq, thread=1), 0, 5)
    _run(round_wq, 5, 19)
    _start(xa_h, xa_v, sem_x.at[0], 0)
    _start(xb_h, xb_v, sem_x.at[1], 0)
    e_s[...] = ((_iota(e_s.shape, 1) >> 4) == _iota(e_s.shape, 0)).astype(F32).astype(BF16)
    o_s[...] = jnp.zeros(o_s.shape, F32)
    cx_s[...] = jnp.zeros(cx_s.shape, F32)
    _run(round_wq, 24, 8)
    _run(round_wu, 0, 24)

    _wait_all(xa_v, sem_x.at[0])
    _wait_all(wqa_v, sem_w.at[0])
    xa = xa_v[...].astype(F32)
    xa = jnp.concatenate([xa, xa], axis=0).astype(BF16)

    def qa_body(j, c):
        w = wqa_v[:, :, pl.ds(pl.multiple_of(j * 1024, 1024), 1024)].reshape(M, 1024)
        qa = _dot(xa, w)
        for h in range(8):
            q_s[8 * j + h] = qa[:, DH * h:DH * (h + 1)]
        _run(round_wu, 24 + 2 * j, 2)
        return c
    lax.fori_loop(0, 4, qa_body, 0)

    _wait_all(xb_v, sem_x.at[1])
    _wait_all(wqb_v, sem_w.at[1])
    xb = xb_v[...].astype(F32)
    xb = jnp.concatenate([jnp.broadcast_to(xb[b:b + 1], (16, M)) for b in range(B)],
                         axis=0).astype(BF16)
    for j in range(4):
        cl_s[j, 0] = xb[:, 128 * j:128 * (j + 1)]
    lhs = _diag16(_dot(xb[:, 512:M], e_s[:64, :1024]))
    qb = tuple(_dot(lhs, wqb_v[8, :, _heads16(g), :].reshape(1024, DH)) for g in range(2))
    _run(round_c, 0, 8)

    def qb_body(j, acc):
        lhs = _diag16(_dot(cl_s[j, 0], e_s[...]))
        out = []
        for g in range(2):
            w = wqb_v[pl.ds(2 * j, 2), :, _heads16(g), :].reshape(2048, DH)
            out.append(acc[g] + _dot(lhs, w))
            _run(round_c, 8 + 6 * j + 3 * g, 3)
        return tuple(out)
    qb = lax.fori_loop(0, 4, qb_body, qb)
    for g in range(2):
        qb_s[g] = qb[g].astype(BF16)

    _wait_all(wuk_v, sem_w.at[2])

    def ql_body(j, c):
        for g in range(2):
            t = _diag16(_dot_nt(qb_s[g], wuk_v[j, :, _heads16(g), :].reshape(2048, DH)))
            _run(round_c, 32 + 8 * j + 4 * g, 2)
            ql_s[j, g] = _dot_nt(t, e_s[...]).astype(BF16)
            _run(round_c, 34 + 8 * j + 4 * g, 2)
        return c
    lax.fori_loop(0, 4, ql_body, 0)

    _run(round_kv0, 0, 4)

    def attn_body(b, c):
        rows = pl.ds(pl.multiple_of(b * 16, 16), 16)
        ql = jnp.concatenate(
            [jnp.concatenate([ql_s[j, g, rows, :] for j in range(4)], axis=1)
             for g in range(2)], axis=0)
        _wait_all(c_v.at[pl.ds(4 * b, 4)], sem_c.at[b])

        def qk(t, m):
            s = _dot_nt(ql, c_v[4 * b + t]) * SCALE
            sb_s[t] = s
            for u in range(8):
                m = jnp.maximum(m, s[:, 128 * u:128 * (u + 1)])
            _run(round_kv0, 4 + 12 * b + 2 * t, 2)
            return m
        m = lax.fori_loop(0, 4, qk, jnp.full((H, 128), -jnp.inf, F32))
        m = jnp.max(m, axis=1, keepdims=True)

        def pv(t, carry):
            l, acc = carry
            p = jnp.exp(sb_s[t] - m)
            acc = acc + _dot(p.astype(BF16), c_v[4 * b + t])
            for u in range(8):
                l = l + p[:, 128 * u:128 * (u + 1)]
            round_kv0(12 + 12 * b + t)
            return l, acc
        l, acc = lax.fori_loop(0, 4, pv, (jnp.zeros((H, 128), F32), jnp.zeros((H, DC), F32)))
        ctx = (acc / jnp.sum(l, axis=1, keepdims=True)).astype(BF16)
        for g in range(2):
            for j in range(4):
                cl_s[j, g, rows, :] = ctx[16 * g:16 * (g + 1), 128 * j:128 * (j + 1)]
        return c
    lax.fori_loop(0, B, attn_body, 0)

    _wait_all(wuv_v, sem_w.at[3])

    def cx_body(j, acc):
        out = []
        for g in range(2):
            lhs = _diag16(_dot(cl_s[j, g], e_s[...]))
            out.append(acc[g] + _dot(lhs, wuv_v[j, :, _heads16(g), :].reshape(2048, DH)))
        _run(round_kv0, 52 + 3 * j, 3)
        return tuple(out)
    cx = lax.fori_loop(0, 4, cx_body, (jnp.zeros((64, DH), F32),) * 2)
    for h in range(H):
        for b in range(B):
            r = 16 * b + h % 16
            cx_s[h, b:b + 1, :] = cx[h // 16][r:r + 1]

    def group(g, c):
        def issue(stage, step):
            def first(n):
                return (0, n[0], n[0] + GH * n[1])[stage] + n[stage] * step

            @pl.when(g < NGRP - 1)
            def _():
                _run(functools.partial(round_kv, g + 1), first(KV_ROUNDS), KV_ROUNDS[stage])

            @pl.when(g == NGRP - 1)
            def _():
                _run(round_wo, first(WO_ROUNDS), WO_ROUNDS[stage])

        slot = g & 1
        batch, h0 = pl.ds(g >> 2, 1), (g & 3) * GH
        issue(0, 0)
        _wait_all(kbuf.at[slot], sem_k.at[slot])

        def qk(i, c):
            q = jnp.broadcast_to(q_s[h0 + i, batch, :], (8, DH)).astype(BF16)
            sa_s[pl.ds(i, 1), :] = _dot_nt(q, kbuf[slot, i])[0:1]
            issue(1, i)
            return c
        lax.fori_loop(0, GH, qk, 0)
        s = sa_s[...] * SCALE
        p = jnp.exp(s - jnp.max(s, axis=1, keepdims=True))
        l = jnp.sum(p, axis=1, keepdims=True)
        sa_s[...] = p
        _wait_all(vbuf.at[slot], sem_v.at[slot])

        def pv(i, acc):
            d = _dot(sa_s[...].astype(BF16), vbuf[slot, i])
            issue(2, i)
            return jnp.where(_iota(d.shape, 0) == i, d, acc)
        o = lax.fori_loop(0, GH, pv, jnp.zeros((GH, DH), F32)) / l
        for i in range(GH):
            o_s[h0 + i, batch, :] = o[i:i + 1]
        return c
    lax.fori_loop(0, NGRP, group, 0)

    oa = jnp.concatenate([o_s[h] for h in range(H)], axis=1).astype(BF16)

    def y_body(j, yb):
        @pl.when(j == 0)
        def _():
            _run(round_wo, WO_EARLY, 64 - WO_EARLY)

        @pl.when(j == 1)
        def _():
            _run(functools.partial(round_wo, last=True), 64, 8)

        def yb_body(i, yb):
            g = 2 * j + i
            _wait_all(wob_v.at[g], sem_ob.at[g])
            for t in range(4):
                yb = yb + _dot_nt(cx_s[g + 8 * t].astype(BF16), wob_v[g, t])
            return yb
        yb = lax.fori_loop(0, 2, yb_body, yb)
        _wait_all(woa_v.at[pl.ds(2 * j, 2)], sem_oa.at[j])
        q_s[j] = _dot_nt(oa, woa_v[pl.ds(2 * j, 2)].reshape(128, H * DH))
        return yb
    yb = lax.fori_loop(0, 4, y_body, jnp.zeros((8, M), F32))
    _wait_all(woa_v.at[8], sem_oa.at[4])
    y = [q_s[j] for j in range(4)] + [_dot_nt(oa, woa_v[8]), yb]
    out_ref[...] = jnp.concatenate(y, axis=1)[0:B].astype(out_ref.dtype)


def _kernel(*refs):
    sems = [pltpu.SemaphoreType.DMA((n,)) for n in (2, 2, 2, 4, B, 5, 8)]
    pl.run_scoped(functools.partial(_stream, *refs), *sems)


@jax.jit
def pallas_concat_heads__mha_block_cached__compressed_kv_cla__decode_kernel(
    A_x: jax.Array,
    A_k_cache: jax.Array,
    A_v_cache: jax.Array,
    A_wq: jax.Array,
    A_wo: jax.Array,
    B_x: jax.Array,
    B_c_kv: jax.Array,
    B_w_q: jax.Array,
    B_w_uk: jax.Array,
    B_w_uv: jax.Array,
    B_w_o: jax.Array,
):
    out = pl.pallas_call(
        _kernel,
        in_specs=[pl.BlockSpec(memory_space=pl.ANY)] * 11,
        out_specs=pl.BlockSpec(memory_space=pltpu.VMEM),
        out_shape=jax.ShapeDtypeStruct((B, 2 * M), BF16),
        scratch_shapes=[
            pltpu.VMEM((B, M), BF16),
            pltpu.VMEM((B, M), BF16),
            pltpu.VMEM((2, GH, S, DH), BF16),
            pltpu.VMEM((2, GH, S, DH), BF16),
            pltpu.VMEM((9, 64, H * DH), BF16),
            pltpu.VMEM((9, 64, H * DH), BF16),
            pltpu.VMEM((16, 1024, DC), BF16),
            pltpu.VMEM((9, 64, H, DH), BF16),
            pltpu.VMEM((4, 128, H, DH), BF16),
            pltpu.VMEM((4, 128, H, DH), BF16),
            pltpu.VMEM((8, 4, M, DH), BF16),
            pltpu.VMEM((H, 8, DH), F32),
            pltpu.VMEM((H, 8, DH), F32),
            pltpu.VMEM((GH, S), F32),
            pltpu.VMEM((128, 2048), BF16),
            pltpu.VMEM((2, 64, DH), BF16),
            pltpu.VMEM((4, 2, 64, 128), BF16),
            pltpu.VMEM((4, H, 1024), F32),
            pltpu.VMEM((4, 2, 64, 128), BF16),
            pltpu.VMEM((H, 8, DH), F32),
        ],
        compiler_params=pltpu.CompilerParams(vmem_limit_bytes=100 * 1024 * 1024),
    )(
        A_x.reshape(B, M),
        A_k_cache.reshape(NGRP, GH, S, DH),
        A_v_cache.reshape(NGRP, GH, S, DH),
        A_wq.reshape(9, 64, H * DH),
        A_wo.T.reshape(9, 64, H * DH),
        B_x.reshape(B, M),
        B_c_kv.reshape(16, 1024, DC),
        B_w_q.reshape(9, 64, H, DH),
        B_w_uk.reshape(4, 128, H, DH),
        B_w_uv.reshape(4, 128, H, DH),
        B_w_o.transpose(0, 2, 1).reshape(4, 8, M, DH),
    )
    return out.reshape(B, 1, 2 * M)
```
